```python
import os as _os
_os.environ.setdefault("JAX_PLATFORMS", "cpu")
import jax
import jax.numpy as jnp

def _softmax(x, axis=-1):
    return jax.nn.softmax(x, axis=axis)
def _gelu(x):
    return jax.nn.gelu(x, approximate=True)
def _silu(x):
    return jax.nn.silu(x)
def _sigmoid(x):
    return jax.nn.sigmoid(x)
def _layernorm(x, axis=-1, eps=1e-5):
    m = jnp.mean(x, axis=axis, keepdims=True)
    v = jnp.var(x, axis=axis, keepdims=True)
    return (x - m) / jnp.sqrt(v + eps)
def _scatter_add(tgt, idx, src, axis=0):
    return tgt.at[idx].add(src)
def _segment_sum(src, seg, n):
    return jax.ops.segment_sum(src, seg, n)
class _Rng:
    def __init__(self, key):
        self._k = key
    def _next(self):
        self._k, sub = jax.random.split(self._k)
        return sub
    def normal(self, shape):
        return jax.random.normal(self._next(), shape, dtype=jnp.bfloat16)
    def randint(self, lo, hi, shape):
        return jax.random.randint(self._next(), shape, lo, hi, dtype=jnp.int32)
    def uniform(self, shape, lo=0.0, hi=1.0):
        return jax.random.uniform(self._next(), shape, jnp.bfloat16, lo, hi)
    def permutation(self, n):
        return jax.random.permutation(self._next(), n)


kernel_name = 'sequential_preLN__ssm_conv_h3__mixer_s_mlp__prompt'

def setup_inputs():
    _rng = _Rng(jax.random.key(int.from_bytes(__import__("os").urandom(4), "little")))
    _w = (lambda a: (lambda t: t.astype(jnp.bfloat16) if jnp.issubdtype(t.dtype, jnp.floating) else t)(jnp.asarray(a)))
    def _A_setup():
        B, S, D = 1, 2048, 640
        ks = 4
        return {
            "q": _w((lambda *s: _rng.normal(s) * 0.05)(B, S, D)),
            "k": _w((lambda *s: _rng.normal(s) * 0.05)(B, S, D)),
            "v": _w((lambda *s: _rng.normal(s) * 0.05)(B, S, D)),
            "shift_k": _w((lambda *s: _rng.normal(s) * 0.05)(D, ks) * 0.5),
            "ssm_k": _w((lambda *s: _rng.normal(s) * 0.05)(D, S) * (1.0 / S ** 0.5)),
            "ssm_D": _w((lambda *s: _rng.normal(s) * 0.05)(D)),
        }
    _A_in = _A_setup()

    def _B_setup():
        B, S, D, F = 1, 2048, 640, 1728
        return {
            "x":  _w((lambda *s: _rng.normal(s) * 0.05)(B, S, D)),
            "w1": _w((lambda *s: _rng.normal(s) * 0.8)(D, D) * (D ** -0.5)),
            "w2": _w((lambda *s: _rng.normal(s) * 0.8)(D, D) * (D ** -0.5)),
            "w3": _w((lambda *s: _rng.normal(s) * 0.8)(D, F) * (D ** -0.5)),
            "w4": _w((lambda *s: _rng.normal(s) * 0.8)(F, D) * (F ** -0.5)),
        }
    _B_in = _B_setup()

    return {
        "A_q": _A_in["q"],
        "A_k": _A_in["k"],
        "A_v": _A_in["v"],
        "A_shift_k": _A_in["shift_k"],
        "A_ssm_k": _A_in["ssm_k"],
        "A_ssm_D": _A_in["ssm_D"],
        "B_x": _B_in["x"],
        "B_w1": _B_in["w1"],
        "B_w2": _B_in["w2"],
        "B_w3": _B_in["w3"],
        "B_w4": _B_in["w4"],
    }

def reference(A_q, A_k, A_v, A_shift_k, A_ssm_k, A_ssm_D, B_x, B_w1, B_w2, B_w3, B_w4):
    def _A_ref(q, k, v, shift_k, ssm_k, ssm_D):
        B, S, D = q.shape
        ks = shift_k.shape[-1]
        k_pad = jnp.pad(k, ((0, 0), (ks - 1, 0), (0, 0)))
        k_shift = jnp.zeros_like(k)
        for t in range(ks):
            k_shift = k_shift + k_pad[:, t:t + S, :] * shift_k[:, ks - 1 - t][None, None, :]
        kv = k_shift * v
        L = 2 * S
        kv_pad = jnp.pad(kv, ((0, 0), (0, S), (0, 0)))
        kf_pad = jnp.pad(ssm_k, ((0, 0), (0, S)))
        kv_f = (lambda x, axes=(-2,-1): jnp.fft.rfft2(x.astype(jnp.float32), axes=axes))(kv_pad[:, None, :, :], axes=(1, 2))
        kf_f = (lambda x, axes=(-2,-1): jnp.fft.rfft2(x.astype(jnp.float32), axes=axes))(kf_pad[:, None, :], axes=(1, 2))
        kf_f = (lambda x, *d: x.transpose(*d))(kf_f, 1, 2, 0)
        y_f = kv_f * kf_f[None, :, :, :]
        y = (lambda x, s, axes=(-2,-1): jnp.fft.irfft2(x, s=s, axes=axes).astype(jnp.bfloat16))(y_f, (1, L), axes=(1, 2))[:, 0, :S, :]
        y = y + kv * ssm_D[None, None, :]
        return q * y

    def _B_ref(x, w1, w2, w3, w4):
        B, S, D = x.shape
        h = _gelu(_layernorm(x, axis=-1) @ w1)
        c = D // 4
        g0 = jnp.pad(h[:, :, 0*c:1*c], ((0, 0), (1, 0), (0, 0)))[:, :S, :]
        g1 = jnp.pad(h[:, :, 1*c:2*c], ((0, 0), (0, 1), (0, 0)))[:, 1:, :]
        g2 = jnp.pad(h[:, :, 2*c:3*c], ((0, 0), (2, 0), (0, 0)))[:, :S, :]
        g3 = jnp.pad(h[:, :, 3*c:   ], ((0, 0), (0, 2), (0, 0)))[:, 2:, :]
        hs = jnp.concatenate([g0, g1, g2, g3], axis=-1) @ w2
        x1 = x + hs
        h2 = _gelu(_layernorm(x1, axis=-1) @ w3) @ w4
        return x1 + h2

    x = A_q
    h = x + _A_ref(_layernorm(x, axis=-1), A_k, A_v, A_shift_k, A_ssm_k, A_ssm_D)
    h2 = h + _B_ref(_layernorm(h, axis=-1), B_w1, B_w2, B_w3, B_w4)
    return h2
```

```python
import numpy as np
import jax
import jax.numpy as jnp
import jax.experimental.pallas as pl
import jax.experimental.pallas.tpu as pltpu

BLK = 128
NF = 2 * BLK
CH = 16
PAD = 8


def _dft_mats():
    e = np.arange(BLK, dtype=np.float64)
    f = np.arange(BLK, dtype=np.float64) + 0.5
    th = 2.0 * np.pi * np.outer(f, e) / NF
    fwd = np.concatenate([np.cos(th), -np.sin(th)], axis=0)
    n = np.arange(BLK, dtype=np.float64) + BLK
    ti = 2.0 * np.pi * np.outer(n, f) / NF
    inv = np.concatenate([np.cos(ti), -np.sin(ti)], axis=1) / BLK
    return fwd.astype(np.float32), inv.astype(np.float32)


def _ln(x):
    m = jnp.mean(x, axis=-1, keepdims=True)
    xc = x - m
    v = jnp.mean(xc * xc, axis=-1, keepdims=True)
    return xc * jax.lax.rsqrt(v + 1e-5)


def _gelu(x):
    return jax.nn.gelu(x, approximate=True)


def _dot(a, b):
    return jnp.dot(a, b, preferred_element_type=jnp.float32)


@jax.jit
def pallas_sequential_preLN__ssm_conv_h3__mixer_s_mlp__prompt_kernel(
    A_q, A_k, A_v, A_shift_k, A_ssm_k, A_ssm_D, B_x, B_w1, B_w2, B_w3, B_w4,
):
    _, S, D = A_q.shape
    F = B_w3.shape[1]
    ks = A_shift_k.shape[1]
    nb = S // BLK
    grp = D // 4
    fwd_np, inv_np = _dft_mats()

    def kernel(q_ref, k_ref, v_ref, sk_ref, ssmk_ref, sd_ref, w1_ref, w2_ref,
               w3_ref, w4_ref, fwd_ref, inv_ref, o_ref,
               xh, kh, pprev, kbuf, hbuf, xbuf, h1buf, ybuf):
        a = pl.program_id(0)

        @pl.when(a == 0)
        def _():
            kbuf[0:PAD, :] = jnp.zeros((PAD, D), jnp.float32)
            pprev[...] = jnp.zeros(pprev.shape, jnp.float32)
            h1buf[0:PAD, :] = jnp.zeros((PAD, D), jnp.float32)
            h1buf[PAD + S:PAD + S + PAD, :] = jnp.zeros((PAD, D), jnp.float32)

        @pl.when(a < nb)
        def _stage1():
            xq = q_ref[...].astype(jnp.float32)
            qn = _ln(xq)
            kbuf[PAD:PAD + BLK, :] = k_ref[...].astype(jnp.float32)
            sk = sk_ref[...].astype(jnp.float32)
            ksh = kbuf[PAD:PAD + BLK, :] * sk[0:1, :]
            for j in range(1, ks):
                ksh = ksh + kbuf[PAD - j:PAD - j + BLK, :] * sk[j:j + 1, :]
            kbuf[0:PAD, :] = kbuf[BLK:BLK + PAD, :]
            kv = (ksh * v_ref[...].astype(jnp.float32)).astype(jnp.bfloat16)
            fwd = fwd_ref[...]
            xh[a] = _dot(fwd, kv)
            p = jax.lax.dot_general(fwd, ssmk_ref[...], (((1,), (1,)), ((), ())),
                                    preferred_element_type=jnp.float32)
            row = jax.lax.broadcasted_iota(jnp.int32, (BLK, 1), 0)
            sig = jnp.where(row % 2 == 0, 1.0, -1.0).astype(jnp.float32)
            kh[a, 0:BLK, :] = pprev[0:BLK, :] + sig * p[BLK:NF, :]
            kh[a, BLK:NF, :] = pprev[BLK:NF, :] - sig * p[0:BLK, :]
            pprev[...] = p

            for c0 in range(0, BLK, CH):
                def body(c, acc):
                    ar, ai = acc
                    xr = xh[c, c0:c0 + CH, :]
                    xi = xh[c, BLK + c0:BLK + c0 + CH, :]
                    kr = kh[a - c, c0:c0 + CH, :]
                    ki = kh[a - c, BLK + c0:BLK + c0 + CH, :]
                    return (ar + (xr * kr - xi * ki), ai + (xr * ki + xi * kr))
                z = jnp.zeros((CH, D), jnp.float32)
                ar, ai = jax.lax.fori_loop(0, a + 1, body, (z, z))
                ybuf[c0:c0 + CH, :] = ar.astype(jnp.bfloat16)
                ybuf[BLK + c0:BLK + c0 + CH, :] = ai.astype(jnp.bfloat16)
            y = _dot(inv_ref[...], ybuf[...])
            y = y + kv.astype(jnp.float32) * sd_ref[...].astype(jnp.float32)
            h = xq + qn * y
            x = _ln(h)
            r0 = pl.multiple_of(a * BLK, BLK)
            hbuf[pl.ds(r0, BLK), :] = h
            xbuf[pl.ds(r0, BLK), :] = x
            h1 = _gelu(_dot(_ln(x).astype(jnp.bfloat16), w1_ref[...]))
            h1buf[pl.ds(pl.multiple_of(PAD + a * BLK, 8), BLK), :] = h1

        @pl.when(a >= 1)
        def _stage2():
            r0 = pl.multiple_of((a - 1) * BLK, BLK)
            win = h1buf[pl.ds(r0, BLK + 2 * PAD), :]
            lane = jax.lax.broadcasted_iota(jnp.int32, (BLK, D), 1)
            hs = jnp.where(lane < grp, win[PAD - 1:PAD - 1 + BLK],
                 jnp.where(lane < 2 * grp, win[PAD + 1:PAD + 1 + BLK],
                 jnp.where(lane < 3 * grp, win[PAD - 2:PAD - 2 + BLK],
                           win[PAD + 2:PAD + 2 + BLK])))
            x1 = xbuf[pl.ds(r0, BLK), :] + _dot(hs.astype(jnp.bfloat16), w2_ref[...])
            g = _gelu(_dot(_ln(x1).astype(jnp.bfloat16), w3_ref[...]))
            h2 = _dot(g.astype(jnp.bfloat16), w4_ref[...])
            o_ref[...] = (hbuf[pl.ds(r0, BLK), :] + x1 + h2).astype(o_ref.dtype)

    cur = lambda a: (jnp.minimum(a, nb - 1), 0)
    const = lambda a: (0, 0)
    full = lambda shp: pl.BlockSpec(shp, const)
    out = pl.pallas_call(
        kernel,
        grid=(nb + 1,),
        in_specs=[
            pl.BlockSpec((BLK, D), cur), pl.BlockSpec((BLK, D), cur),
            pl.BlockSpec((BLK, D), cur), full((ks, D)),
            pl.BlockSpec((D, BLK), lambda a: (0, jnp.minimum(a, nb - 1))),
            full((1, D)), full((D, D)), full((D, D)), full((D, F)), full((F, D)),
            full((NF, BLK)), full((BLK, NF)),
        ],
        out_specs=pl.BlockSpec((BLK, D), lambda a: (jnp.maximum(a - 1, 0), 0)),
        out_shape=jax.ShapeDtypeStruct((S, D), A_q.dtype),
        scratch_shapes=[
            pltpu.VMEM((nb, NF, D), jnp.float32),
            pltpu.VMEM((nb, NF, D), jnp.float32),
            pltpu.VMEM((NF, D), jnp.float32),
            pltpu.VMEM((PAD + BLK, D), jnp.float32),
            pltpu.VMEM((S, D), jnp.float32),
            pltpu.VMEM((S, D), jnp.float32),
            pltpu.VMEM((S + 2 * PAD, D), jnp.float32),
            pltpu.VMEM((NF, D), jnp.bfloat16),
        ],
        compiler_params=pltpu.CompilerParams(
            dimension_semantics=("arbitrary",),
            vmem_limit_bytes=100 * 1024 * 1024),
    )(A_q[0], A_k[0], A_v[0], A_shift_k.T, A_ssm_k, A_ssm_D.reshape(1, D),
      B_w1, B_w2, B_w3, B_w4,
      jnp.asarray(fwd_np, jnp.bfloat16), jnp.asarray(inv_np, jnp.bfloat16))
    return out[None]
```

```python
import numpy as np
import jax
import jax.numpy as jnp
import jax.experimental.pallas as pl
import jax.experimental.pallas.tpu as pltpu

BLK = 128
NF = 2 * BLK
CH = 8
RB = 256
SUB = RB // BLK
PAD = 8


def _dft_mats():
    e = np.arange(BLK, dtype=np.float64)
    f = np.arange(BLK, dtype=np.float64) + 0.5
    th = 2.0 * np.pi * np.outer(f, e) / NF
    fwd = np.concatenate([np.cos(th), -np.sin(th)], axis=0)
    n = np.arange(BLK, dtype=np.float64) + BLK
    ti = 2.0 * np.pi * np.outer(n, f) / NF
    inv = np.concatenate([np.cos(ti), -np.sin(ti)], axis=1) / BLK
    return fwd.astype(np.float32), inv.astype(np.float32)


def _ln(x):
    m = jnp.mean(x, axis=-1, keepdims=True)
    xc = x - m
    v = jnp.mean(xc * xc, axis=-1, keepdims=True)
    return xc * jax.lax.rsqrt(v + 1e-5)


def _gelu(x):
    return jax.nn.gelu(x, approximate=True)


def _dot(a, b):
    return jnp.dot(a, b, preferred_element_type=jnp.float32)


@jax.jit
def pallas_sequential_preLN__ssm_conv_h3__mixer_s_mlp__prompt_kernel(
    A_q, A_k, A_v, A_shift_k, A_ssm_k, A_ssm_D, B_x, B_w1, B_w2, B_w3, B_w4,
):
    _, S, D = A_q.shape
    F = B_w3.shape[1]
    ks = A_shift_k.shape[1]
    nb = S // BLK
    ns = S // RB
    grp = D // 4
    fwd_np, inv_np = _dft_mats()

    def kernel(q_ref, k_ref, v_ref, sk_ref, ssmk_ref, sd_ref, w1_ref, w2_ref,
               w3_ref, w4_ref, fwd_ref, inv_ref, o_ref,
               xh, kh, pprev, kbuf, hbuf, xbuf, h1buf, ybuf):
        a = pl.program_id(0)

        @pl.when(a == 0)
        def _():
            kbuf[0:PAD, :] = jnp.zeros((PAD, D), jnp.float32)
            pprev[...] = jnp.zeros(pprev.shape, jnp.float32)
            h1buf[0:PAD, :] = jnp.zeros((PAD, D), jnp.float32)
            h1buf[PAD + S:PAD + S + PAD, :] = jnp.zeros((PAD, D), jnp.float32)

        @pl.when(a < ns)
        def _stage1():
            xq = q_ref[...].astype(jnp.float32)
            qn = _ln(xq)
            kbuf[PAD:PAD + RB, :] = k_ref[...].astype(jnp.float32)
            sk = sk_ref[...].astype(jnp.float32)
            ksh = kbuf[PAD:PAD + RB, :] * sk[0:1, :]
            for j in range(1, ks):
                ksh = ksh + kbuf[PAD - j:PAD - j + RB, :] * sk[j:j + 1, :]
            kbuf[0:PAD, :] = kbuf[RB:RB + PAD, :]
            kv = (ksh * v_ref[...].astype(jnp.float32)).astype(jnp.bfloat16)
            fwd = fwd_ref[...]
            row = jax.lax.broadcasted_iota(jnp.int32, (BLK, 1), 0)
            sig = jnp.where(row % 2 == 0, 1.0, -1.0).astype(jnp.float32)
            ys = []
            for sub in range(SUB):
                aa = a * SUB + sub
                xh[aa] = _dot(fwd, kv[sub * BLK:(sub + 1) * BLK, :])
                p = jax.lax.dot_general(fwd, ssmk_ref[:, sub * BLK:(sub + 1) * BLK],
                                        (((1,), (1,)), ((), ())),
                                        preferred_element_type=jnp.float32)
                kh[aa, 0:BLK, :] = pprev[0:BLK, :] + sig * p[BLK:NF, :]
                kh[aa, BLK:NF, :] = pprev[BLK:NF, :] - sig * p[0:BLK, :]
                pprev[...] = p
                for c0 in range(0, BLK, CH):
                    def body(c, acc, aa=aa, c0=c0):
                        ar, ai = acc
                        xr = xh[c, c0:c0 + CH, :]
                        xi = xh[c, BLK + c0:BLK + c0 + CH, :]
                        kr = kh[aa - c, c0:c0 + CH, :]
                        ki = kh[aa - c, BLK + c0:BLK + c0 + CH, :]
                        return (ar + (xr * kr - xi * ki), ai + (xr * ki + xi * kr))
                    z = jnp.zeros((CH, D), jnp.float32)
                    ar, ai = jax.lax.fori_loop(0, aa + 1, body, (z, z))
                    ybuf[c0:c0 + CH, :] = ar.astype(jnp.bfloat16)
                    ybuf[BLK + c0:BLK + c0 + CH, :] = ai.astype(jnp.bfloat16)
                ys.append(_dot(inv_ref[...], ybuf[...]))
            y = jnp.concatenate(ys, axis=0)
            y = y + kv.astype(jnp.float32) * sd_ref[...].astype(jnp.float32)
            h = xq + qn * y
            x = _ln(h)
            r0 = pl.multiple_of(a * RB, RB)
            hbuf[pl.ds(r0, RB), :] = h
            xbuf[pl.ds(r0, RB), :] = x
            h1 = _gelu(_dot(_ln(x).astype(jnp.bfloat16), w1_ref[...]))
            h1buf[pl.ds(pl.multiple_of(PAD + a * RB, 8), RB), :] = h1

        @pl.when(a >= 1)
        def _stage2():
            r0 = pl.multiple_of((a - 1) * RB, RB)
            win = h1buf[pl.ds(r0, RB + 2 * PAD), :]
            lane = jax.lax.broadcasted_iota(jnp.int32, (RB, D), 1)
            hs = jnp.where(lane < grp, win[PAD - 1:PAD - 1 + RB],
                 jnp.where(lane < 2 * grp, win[PAD + 1:PAD + 1 + RB],
                 jnp.where(lane < 3 * grp, win[PAD - 2:PAD - 2 + RB],
                           win[PAD + 2:PAD + 2 + RB])))
            x1 = xbuf[pl.ds(r0, RB), :] + _dot(hs.astype(jnp.bfloat16), w2_ref[...])
            g = _gelu(_dot(_ln(x1).astype(jnp.bfloat16), w3_ref[...]))
            h2 = _dot(g.astype(jnp.bfloat16), w4_ref[...])
            o_ref[...] = (hbuf[pl.ds(r0, RB), :] + x1 + h2).astype(o_ref.dtype)

    cur = lambda a: (jnp.minimum(a, ns - 1), 0)
    const = lambda a: (0, 0)
    full = lambda shp: pl.BlockSpec(shp, const)
    out = pl.pallas_call(
        kernel,
        grid=(ns + 1,),
        in_specs=[
            pl.BlockSpec((RB, D), cur), pl.BlockSpec((RB, D), cur),
            pl.BlockSpec((RB, D), cur), full((ks, D)),
            pl.BlockSpec((D, RB), lambda a: (0, jnp.minimum(a, ns - 1))),
            full((1, D)), full((D, D)), full((D, D)), full((D, F)), full((F, D)),
            full((NF, BLK)), full((BLK, NF)),
        ],
        out_specs=pl.BlockSpec((RB, D), lambda a: (jnp.maximum(a - 1, 0), 0)),
        out_shape=jax.ShapeDtypeStruct((S, D), A_q.dtype),
        scratch_shapes=[
            pltpu.VMEM((nb, NF, D), jnp.float32),
            pltpu.VMEM((nb, NF, D), jnp.float32),
            pltpu.VMEM((NF, D), jnp.float32),
            pltpu.VMEM((PAD + RB, D), jnp.float32),
            pltpu.VMEM((S, D), jnp.float32),
            pltpu.VMEM((S, D), jnp.float32),
            pltpu.VMEM((S + 2 * PAD, D), jnp.float32),
            pltpu.VMEM((NF, D), jnp.bfloat16),
        ],
        compiler_params=pltpu.CompilerParams(
            dimension_semantics=("arbitrary",),
            vmem_limit_bytes=100 * 1024 * 1024),
    )(A_q[0], A_k[0], A_v[0], A_shift_k.T, A_ssm_k, A_ssm_D.reshape(1, D),
      B_w1, B_w2, B_w3, B_w4,
      jnp.asarray(fwd_np, jnp.bfloat16), jnp.asarray(inv_np, jnp.bfloat16))
    return out[None]
```
